```python
import jax
import jax.numpy as jnp

def _softmax(x, axis=-1):
    return jax.nn.softmax(x, axis=axis)
def _gelu(x):
    return jax.nn.gelu(x, approximate=True)
def _silu(x):
    return jax.nn.silu(x)
def _sigmoid(x):
    return jax.nn.sigmoid(x)
def _layernorm(x, axis=-1, eps=1e-5):
    m = jnp.mean(x, axis=axis, keepdims=True)
    v = jnp.var(x, axis=axis, keepdims=True)
    return (x - m) / jnp.sqrt(v + eps)
def _scatter_add(tgt, idx, src, axis=0):
    return tgt.at[idx].add(src)
def _segment_sum(src, seg, n):
    return jax.ops.segment_sum(src, seg, n)
class _Rng:
    def __init__(self, key):
        self._k = key
    def _next(self):
        self._k, sub = jax.random.split(self._k)
        return sub
    def normal(self, shape):
        return jax.random.normal(self._next(), shape, dtype=jnp.bfloat16)
    def randint(self, lo, hi, shape):
        return jax.random.randint(self._next(), shape, lo, hi, dtype=jnp.int32)
    def uniform(self, shape, lo=0.0, hi=1.0):
        return jax.random.uniform(self._next(), shape, jnp.bfloat16, lo, hi)
    def permutation(self, n):
        return jax.random.permutation(self._next(), n)


kernel_name = 'gated_mix__sliding_local_dilated__glu_gated_reglu__prompt'

def setup_inputs():
    _rng = _Rng(jax.random.key(int.from_bytes(__import__("os").urandom(4), "little")))
    _w = (lambda a: (lambda t: t.astype(jnp.bfloat16) if jnp.issubdtype(t.dtype, jnp.floating) else t)(jnp.asarray(a)))
    def _A_setup():
        B, S, D = 1, 2048, 1024
        return {
            "x": _w((lambda *s: _rng.normal(s) * 0.05)(B, S, D)),
            "wqkv": _w((lambda *s: _rng.normal(s) * 0.05)(D, 3 * D)),
            "wo": _w((lambda *s: _rng.normal(s) * 0.05)(D, D)),
        }
    _A_in = _A_setup()

    def _B_setup():
        B, S, D, F = 1, 2048, 1024, 3584
        return {
            "x": _w((lambda *s: _rng.normal(s) * 0.05)(B, S, D)),
            "W_gate": _w((lambda *s: _rng.normal(s) * 0.05)(D, F) * (2.0 / D) ** 0.5),
            "W_up": _w((lambda *s: _rng.normal(s) * 0.05)(D, F) * (2.0 / D) ** 0.5),
            "W_down": _w((lambda *s: _rng.normal(s) * 0.05)(F, D) * (1.0 / F) ** 0.5),
        }
    _B_in = _B_setup()

    return {
        "A_x": _A_in["x"],
        "A_wqkv": _A_in["wqkv"],
        "A_wo": _A_in["wo"],
        "B_x": _B_in["x"],
        "B_W_gate": _B_in["W_gate"],
        "B_W_up": _B_in["W_up"],
        "B_W_down": _B_in["W_down"],
        "gate_w": _w((lambda *s: _rng.normal(s) * 0.05)(1024)),
    }

def reference(A_x, A_wqkv, A_wo, B_x, B_W_gate, B_W_up, B_W_down, gate_w):
    def _A_ref(x, wqkv, wo):
        B, S, D = x.shape
        H = 32; Dh = D // H
        W, dil = 8, 2
        qkv = (lambda x, *d: x.transpose(*d))((x @ wqkv).reshape(B, S, 3, H, Dh), 2, 0, 3, 1, 4)
        q, k, v = qkv[0], qkv[1], qkv[2]
        scale = Dh ** -0.5
        pos = jnp.arange(S)
        off = jnp.arange(W) * dil
        idx = pos[:, None] - off[None, :]
        mask = idx >= 0
        idx_c = jnp.where(mask, idx, 0).reshape(-1)
        kg = k[:, :, idx_c, :].reshape(B, H, S, W, Dh)
        vg = v[:, :, idx_c, :].reshape(B, H, S, W, Dh)
        logits = jnp.einsum("bhsd,bhswd->bhsw", q, kg) * scale
        logits = jnp.where(mask[None, None, :, :], logits, -1e9)
        attn = _softmax(logits, axis=-1)
        o = jnp.einsum("bhsw,bhswd->bhsd", attn, vg)
        return (lambda x, *d: x.transpose(*d))(o, 0, 2, 1, 3).reshape(B, S, D) @ wo

    def _B_ref(x, W_gate, W_up, W_down):
        gate = jnp.einsum("bsd,df->bsf", x, W_gate)
        up = jnp.einsum("bsd,df->bsf", x, W_up)
        gate = gate * (lambda x, dt: x.astype(dt))(gate > 0, gate.dtype)
        h = gate * up
        return jnp.einsum("bsf,fd->bsd", h, W_down)

    x = A_x
    g = _sigmoid((x * gate_w).sum(-1, keepdims=True))
    a = _A_ref(x, A_wqkv, A_wo)
    b = _B_ref(x, B_W_gate, B_W_up, B_W_down)
    return g * a + (1 - g) * b
```

```python
import functools

import jax
import jax.numpy as jnp
import numpy as np
import jax.experimental.pallas as pl
import jax.experimental.pallas.tpu as pltpu

_H = 32
_W = 8
_DIL = 2
_HALO = 16
_TS = 512
_FC = 512


def _kernel(x_ref, gw_ref, wqkv_hbm, wo_hbm, wg_hbm, wu_hbm, wd_hbm, o_ref,
            wqkv_v, wo_v, wg_v, wu_v, wd_v, k_s, v_s, o_s, sem_a, sem_f,
            *, ts, fc, nf, d):
    i = pl.program_id(0)
    nch = d // 128

    def ffn_copies(j):
        return (
            pltpu.make_async_copy(wg_hbm.at[:, pl.ds(j * fc, fc)], wg_v.at[j], sem_f.at[0, j]),
            pltpu.make_async_copy(wu_hbm.at[:, pl.ds(j * fc, fc)], wu_v.at[j], sem_f.at[1, j]),
            pltpu.make_async_copy(wd_hbm.at[pl.ds(j * fc, fc), :], wd_v.at[j], sem_f.at[2, j]),
        )

    def att_copies():
        return (
            pltpu.make_async_copy(wqkv_hbm, wqkv_v, sem_a.at[0]),
            pltpu.make_async_copy(wo_hbm, wo_v, sem_a.at[1]),
        )

    @pl.when(i == 0)
    def _():
        for j in range(nf):
            for c in ffn_copies(j):
                c.start()
        for c in att_copies():
            c.start()
        k_s[:, pl.ds(ts, _HALO), :] = jnp.zeros((nch, _HALO, 128), jnp.float32)
        v_s[:, pl.ds(ts, _HALO), :] = jnp.zeros((nch, _HALO, 128), jnp.float32)

    x = x_ref[...]

    acc = None
    for j in range(nf):
        @pl.when(i == 0)
        def _():
            for c in ffn_copies(j):
                c.wait()
        gate = jnp.dot(x, wg_v[j], preferred_element_type=jnp.float32)
        up = jnp.dot(x, wu_v[j], preferred_element_type=jnp.float32)
        h = ((gate * (gate > 0).astype(jnp.float32)) * up).astype(jnp.bfloat16)
        part = jnp.dot(h, wd_v[j], preferred_element_type=jnp.float32)
        acc = part if acc is None else acc + part

    @pl.when(i == 0)
    def _():
        for c in att_copies():
            c.wait()

    scale = np.float32((d // _H) ** -0.5)
    qkv = jnp.dot(x, wqkv_v[...], preferred_element_type=jnp.float32)
    k_s[:, pl.ds(0, _HALO), :] = k_s[:, pl.ds(ts, _HALO), :]
    v_s[:, pl.ds(0, _HALO), :] = v_s[:, pl.ds(ts, _HALO), :]
    for c in range(nch):
        k_s[c, pl.ds(_HALO, ts), :] = qkv[:, d + c * 128: d + (c + 1) * 128]
        v_s[c, pl.ds(_HALO, ts), :] = qkv[:, 2 * d + c * 128: 2 * d + (c + 1) * 128]

    row = i * ts + jax.lax.broadcasted_iota(jnp.int32, (ts, 128), 0)
    logits = []
    for w in range(_W):
        s = None
        for c in range(nch):
            p = qkv[:, c * 128:(c + 1) * 128] * k_s[c, pl.ds(_HALO - _DIL * w, ts), :]
            s = p if s is None else s + p
        s = s + pltpu.roll(s, 64, 1)
        s = s + pltpu.roll(s, 32, 1)
        l = s * scale
        if w > 0:
            l = jnp.where(row >= _DIL * w, l, np.float32(-1e9))
        logits.append(l)
    m = functools.reduce(jnp.maximum, logits)
    es = [jnp.exp(l - m) for l in logits]
    den = functools.reduce(lambda a, b: a + b, es)
    inv = 1.0 / den
    ps = [e * inv for e in es]
    for c in range(nch):
        o = None
        for w in range(_W):
            t = ps[w] * v_s[c, pl.ds(_HALO - _DIL * w, ts), :]
            o = t if o is None else o + t
        o_s[:, c * 128:(c + 1) * 128] = o.astype(jnp.bfloat16)
    a = jnp.dot(o_s[...], wo_v[...], preferred_element_type=jnp.float32)

    xf = x.astype(jnp.float32) * gw_ref[...].astype(jnp.float32)
    g = jax.nn.sigmoid(jnp.sum(xf, axis=-1, keepdims=True))
    o_ref[...] = (g * a + (1.0 - g) * acc).astype(o_ref.dtype)


@jax.jit
def pallas_gated_mix__sliding_local_dilated__glu_gated_reglu__prompt_kernel(
    A_x: jax.Array,
    A_wqkv: jax.Array,
    A_wo: jax.Array,
    B_x: jax.Array,
    B_W_gate: jax.Array,
    B_W_up: jax.Array,
    B_W_down: jax.Array,
    gate_w: jax.Array,
):
    del B_x
    B, S, D = A_x.shape
    F = B_W_gate.shape[1]
    Dh = D // _H
    ts, fc = _TS, _FC
    nf = F // fc
    nch = D // 128
    x2 = A_x.reshape(B * S, D)
    wqkv = A_wqkv.reshape(D, 3, _H, Dh).transpose(0, 1, 3, 2).reshape(D, 3 * D)
    wo = A_wo.reshape(_H, Dh, D).transpose(1, 0, 2).reshape(D, D)
    gw = gate_w.reshape(1, D)

    any_spec = pl.BlockSpec(memory_space=pl.ANY)
    out = pl.pallas_call(
        functools.partial(_kernel, ts=ts, fc=fc, nf=nf, d=D),
        grid=(B * S // ts,),
        in_specs=[
            pl.BlockSpec((ts, D), lambda i: (i, 0)),
            pl.BlockSpec((1, D), lambda i: (0, 0)),
            any_spec, any_spec, any_spec, any_spec, any_spec,
        ],
        out_specs=pl.BlockSpec((ts, D), lambda i: (i, 0)),
        out_shape=jax.ShapeDtypeStruct((B * S, D), A_x.dtype),
        scratch_shapes=[
            pltpu.VMEM((D, 3 * D), jnp.bfloat16),
            pltpu.VMEM((D, D), jnp.bfloat16),
            pltpu.VMEM((nf, D, fc), jnp.bfloat16),
            pltpu.VMEM((nf, D, fc), jnp.bfloat16),
            pltpu.VMEM((nf, fc, D), jnp.bfloat16),
            pltpu.VMEM((nch, ts + _HALO, 128), jnp.float32),
            pltpu.VMEM((nch, ts + _HALO, 128), jnp.float32),
            pltpu.VMEM((ts, D), jnp.bfloat16),
            pltpu.SemaphoreType.DMA((2,)),
            pltpu.SemaphoreType.DMA((3, nf)),
        ],
        compiler_params=pltpu.CompilerParams(
            dimension_semantics=("arbitrary",),
            vmem_limit_bytes=110 * 1024 * 1024,
        ),
    )(x2, gw, wqkv, wo, B_W_gate, B_W_up, B_W_down)
    return out.reshape(B, S, D)
```

```python
import functools

import jax
import jax.numpy as jnp
import numpy as np
import jax.experimental.pallas as pl
import jax.experimental.pallas.tpu as pltpu

_H = 32
_W = 8
_DIL = 2
_HALO = 16
_FLAGS = {"XLA_TPU_EVENLY_DISTRIBUTE_CRITICAL_NODES": True}
_TF = 512
_TA = 512
_FC = 512


def _kernel(x_hbm, gw_ref, wqkv_hbm, wo_hbm, wg_hbm, wu_hbm, wd_hbm, o_hbm,
            x_v, wqkv_v, wo_v, wg_v, wu_v, wd_v, acc_s, k_s, v_s, a_s, out_v, t_s, u_s,
            sem_x, sem_a, sem_f, sem_o, *, S, d, tf, ta, fc, nf):
    nch = d // 128
    nrf = S // tf
    nra = S // ta
    f32 = jnp.float32

    def x_copy(r):
        return pltpu.make_async_copy(x_hbm.at[pl.ds(r * tf, tf), :],
                                     x_v.at[pl.ds(r * tf, tf), :], sem_x.at[r])

    def ffn_copies(j):
        return (
            pltpu.make_async_copy(wg_hbm.at[:, pl.ds(j * fc, fc)], wg_v.at[j], sem_f.at[0, j]),
            pltpu.make_async_copy(wu_hbm.at[:, pl.ds(j * fc, fc)], wu_v.at[j], sem_f.at[1, j]),
            pltpu.make_async_copy(wd_hbm.at[pl.ds(j * fc, fc), :], wd_v.at[j], sem_f.at[2, j]),
        )

    att_copies = (
        pltpu.make_async_copy(wqkv_hbm, wqkv_v, sem_a.at[0]),
        pltpu.make_async_copy(wo_hbm, wo_v, sem_a.at[1]),
    )

    def out_copy(r):
        return pltpu.make_async_copy(out_v.at[pl.ds(r * ta, ta), :],
                                     o_hbm.at[pl.ds(r * ta, ta), :], sem_o.at[r])

    x_copy(0).start()
    for c in ffn_copies(0):
        c.start()

    def ffn_tile(j, r, first):
        rows = pl.ds(pl.multiple_of(r * tf, tf), tf)
        x = x_v[rows, :]
        gate = jnp.dot(x, wg_v[j], preferred_element_type=f32)
        up = jnp.dot(x, wu_v[j], preferred_element_type=f32)
        h = ((gate * (gate > 0).astype(f32)) * up).astype(jnp.bfloat16)
        part = jnp.dot(h, wd_v[j], preferred_element_type=f32)
        if first:
            acc_s[rows, :] = part
        else:
            acc_s[rows, :] += part

    x_copy(0).wait()
    for c in ffn_copies(0):
        c.wait()
    for r in range(1, nrf):
        x_copy(r).start()
    for c in ffn_copies(1):
        c.start()
    k_s[:, pl.ds(0, _HALO), :] = jnp.zeros((nch, _HALO, 128), f32)
    v_s[:, pl.ds(0, _HALO), :] = jnp.zeros((nch, _HALO, 128), f32)

    def first_body(r, carry):
        @pl.when(r > 0)
        def _():
            x_copy(r).wait()
        ffn_tile(0, r, True)
        return carry
    jax.lax.fori_loop(0, nrf, first_body, 0)

    def chunk_body(j, carry):
        for c in ffn_copies(j):
            c.wait()

        @pl.when(j + 1 < nf)
        def _():
            for c in ffn_copies(j + 1):
                c.start()

        @pl.when(j == 2)
        def _():
            att_copies[0].start()

        @pl.when(j == 3)
        def _():
            att_copies[1].start()

        def row_body(r, carry2):
            ffn_tile(j, r, False)
            return carry2
        return jax.lax.fori_loop(0, nrf, row_body, carry)
    jax.lax.fori_loop(1, nf - 1, chunk_body, 0)

    for c in ffn_copies(nf - 1) + att_copies:
        c.wait()
    dh = d // _H
    wr = d // 2 // nrf
    wc = d // nrf

    def last_body(r, carry):
        ffn_tile(nf - 1, r, False)
        for b in range(wr // 128):
            rows_b = pl.ds(pl.multiple_of(r * (2 * wr) + b * 256, 256), 256)
            words = pltpu.bitcast(wqkv_v[rows_b, :], jnp.int32)
            t_s[b] = words.T
            parts = [t_s[b, pl.ds(m * d + e, _H, stride=dh), :]
                     for m in range(3) for e in range(dh)]
            wqkv_v[rows_b, :] = pltpu.bitcast(jnp.concatenate(parts, axis=0).T, jnp.bfloat16)
        for b in range(wc // 128):
            cols = pl.ds(pl.multiple_of(r * wc + b * 128, 128), 128)
            u_s[b] = wo_v[:, cols].astype(f32)
            parts = [u_s[b, pl.ds(e, _H, stride=dh), :] for e in range(dh)]
            wo_v[:, cols] = jnp.concatenate(parts, axis=0).astype(jnp.bfloat16)
        return carry
    jax.lax.fori_loop(0, nrf, last_body, 0)

    scale = np.float32((d // _H) ** -0.5)
    gw = gw_ref[...].astype(f32)

    def att_body(r, carry):
        r0 = pl.multiple_of(r * ta, ta)
        rows = pl.ds(r0, ta)
        x = x_v[rows, :]
        qkv = jnp.dot(x, wqkv_v[...], preferred_element_type=f32)
        for c in range(nch):
            k_s[c, pl.ds(_HALO, ta), :] = qkv[:, d + c * 128: d + (c + 1) * 128]
            v_s[c, pl.ds(_HALO, ta), :] = qkv[:, 2 * d + c * 128: 2 * d + (c + 1) * 128]

        row = r0 + jax.lax.broadcasted_iota(jnp.int32, (ta, 128), 0)
        logits = []
        for w in range(_W):
            s = None
            for c in range(nch):
                p = qkv[:, c * 128:(c + 1) * 128] * k_s[c, pl.ds(_HALO - _DIL * w, ta), :]
                s = p if s is None else s + p
            s = s + pltpu.roll(s, 64, 1)
            s = s + pltpu.roll(s, 32, 1)
            l = s * scale
            if w > 0:
                l = jnp.where(row >= _DIL * w, l, np.float32(-1e9))
            logits.append(l)
        m = functools.reduce(jnp.maximum, logits)
        es = [jnp.exp(l - m) for l in logits]
        den = functools.reduce(lambda a, b: a + b, es)
        inv = 1.0 / den
        ps = [e * inv for e in es]
        for c in range(nch):
            o = None
            for w in range(_W):
                t = ps[w] * v_s[c, pl.ds(_HALO - _DIL * w, ta), :]
                o = t if o is None else o + t
            a_s[:, c * 128:(c + 1) * 128] = o.astype(jnp.bfloat16)
        k_s[:, pl.ds(0, _HALO), :] = k_s[:, pl.ds(ta, _HALO), :]
        v_s[:, pl.ds(0, _HALO), :] = v_s[:, pl.ds(ta, _HALO), :]
        a = jnp.dot(a_s[...], wo_v[...], preferred_element_type=f32)

        g = jax.nn.sigmoid(jnp.sum(x.astype(f32) * gw, axis=-1, keepdims=True))
        out_v[rows, :] = (g * a + (1.0 - g) * acc_s[rows, :]).astype(out_v.dtype)
        out_copy(r).start()
        return carry
    jax.lax.fori_loop(0, nra, att_body, 0)
    for r in range(nra):
        out_copy(r).wait()


@jax.jit
def pallas_gated_mix__sliding_local_dilated__glu_gated_reglu__prompt_kernel(
    A_x: jax.Array,
    A_wqkv: jax.Array,
    A_wo: jax.Array,
    B_x: jax.Array,
    B_W_gate: jax.Array,
    B_W_up: jax.Array,
    B_W_down: jax.Array,
    gate_w: jax.Array,
):
    del B_x
    B, S, D = A_x.shape
    F = B_W_gate.shape[1]
    tf, ta, fc = _TF, _TA, _FC
    nf = F // fc
    nch = D // 128
    x2 = A_x.reshape(B * S, D)
    gw = gate_w.reshape(1, D)

    any_spec = pl.BlockSpec(memory_space=pl.ANY)
    bf16 = jnp.bfloat16
    out = pl.pallas_call(
        functools.partial(_kernel, S=S, d=D, tf=tf, ta=ta, fc=fc, nf=nf),
        in_specs=[
            any_spec,
            pl.BlockSpec(memory_space=pltpu.VMEM),
            any_spec, any_spec, any_spec, any_spec, any_spec,
        ],
        out_specs=any_spec,
        out_shape=jax.ShapeDtypeStruct((S, D), A_x.dtype),
        scratch_shapes=[
            pltpu.VMEM((S, D), bf16),
            pltpu.VMEM((D, 3 * D), bf16),
            pltpu.VMEM((D, D), bf16),
            pltpu.VMEM((nf, D, fc), bf16),
            pltpu.VMEM((nf, D, fc), bf16),
            pltpu.VMEM((nf, fc, D), bf16),
            pltpu.VMEM((S, D), jnp.float32),
            pltpu.VMEM((nch, ta + _HALO, 128), jnp.float32),
            pltpu.VMEM((nch, ta + _HALO, 128), jnp.float32),
            pltpu.VMEM((ta, D), bf16),
            pltpu.VMEM((S, D), A_x.dtype),
            pltpu.VMEM((D // 2 // (S // tf) // 128, 3 * D, 128), jnp.int32),
            pltpu.VMEM((D // (S // tf) // 128, D, 128), jnp.float32),
            pltpu.SemaphoreType.DMA((S // tf,)),
            pltpu.SemaphoreType.DMA((2,)),
            pltpu.SemaphoreType.DMA((3, nf)),
            pltpu.SemaphoreType.DMA((S // ta,)),
        ],
        compiler_params=pltpu.CompilerParams(
            vmem_limit_bytes=110 * 1024 * 1024,
            flags=_FLAGS,
        ),
    )(x2, gw, A_wqkv, A_wo, B_W_gate, B_W_up, B_W_down)
    return out.reshape(B, S, D)
```

```python
import functools

import jax
import jax.numpy as jnp
import numpy as np
import jax.experimental.pallas as pl
import jax.experimental.pallas.tpu as pltpu

_H = 32
_W = 8
_DIL = 2
_HALO = 16
_FLAGS = {"XLA_TPU_EVENLY_DISTRIBUTE_CRITICAL_NODES": True}
_RG = 16
_RGV = 64
_TF = 512
_TA = 512
_FC = 512


def _kernel(x_hbm, gw_ref, wqkv_hbm, wo_hbm, wg_hbm, wu_hbm, wd_hbm, o_hbm,
            x_v, wqkv_v, wo_v, wg_v, wu_v, wd_v, acc_s, k_s, v_s, q_s, p_s, a_s, out_v, t_s, u_s,
            sem_x, sem_a, sem_f, sem_o, *, S, d, tf, ta, fc, nf):
    nch = d // 128
    nrf = S // tf
    nra = S // ta
    f32 = jnp.float32

    def x_copy(r):
        return pltpu.make_async_copy(x_hbm.at[pl.ds(r * tf, tf), :],
                                     x_v.at[pl.ds(r * tf, tf), :], sem_x.at[r])

    def ffn_copies(j):
        return (
            pltpu.make_async_copy(wg_hbm.at[:, pl.ds(j * fc, fc)], wg_v.at[j], sem_f.at[0, j]),
            pltpu.make_async_copy(wu_hbm.at[:, pl.ds(j * fc, fc)], wu_v.at[j], sem_f.at[1, j]),
            pltpu.make_async_copy(wd_hbm.at[pl.ds(j * fc, fc), :], wd_v.at[j], sem_f.at[2, j]),
        )

    att_copies = (
        pltpu.make_async_copy(wqkv_hbm, wqkv_v, sem_a.at[0]),
        pltpu.make_async_copy(wo_hbm, wo_v, sem_a.at[1]),
    )

    def out_copy(r):
        return pltpu.make_async_copy(out_v.at[pl.ds(r * ta, ta), :],
                                     o_hbm.at[pl.ds(r * ta, ta), :], sem_o.at[r])

    x_copy(0).start()
    for c in ffn_copies(0):
        c.start()

    def ffn_tile(j, r, first):
        rows = pl.ds(pl.multiple_of(r * tf, tf), tf)
        x = x_v[rows, :]
        gate = jnp.dot(x, wg_v[j], preferred_element_type=f32)
        up = jnp.dot(x, wu_v[j], preferred_element_type=f32)
        h = ((gate * (gate > 0).astype(f32)) * up).astype(jnp.bfloat16)
        part = jnp.dot(h, wd_v[j], preferred_element_type=f32)
        if first:
            acc_s[rows, :] = part
        else:
            acc_s[rows, :] += part

    x_copy(0).wait()
    for c in ffn_copies(0):
        c.wait()
    for r in range(1, nrf):
        x_copy(r).start()
    for c in ffn_copies(1):
        c.start()
    k_s[:, pl.ds(0, _HALO), :] = jnp.zeros((nch, _HALO, 128), f32)
    v_s[:, pl.ds(0, _HALO), :] = jnp.zeros((nch, _HALO, 128), f32)

    def first_body(r, carry):
        @pl.when(r > 0)
        def _():
            x_copy(r).wait()
        ffn_tile(0, r, True)
        return carry
    jax.lax.fori_loop(0, nrf, first_body, 0)

    def chunk_body(j, carry):
        for c in ffn_copies(j):
            c.wait()

        @pl.when(j + 1 < nf)
        def _():
            for c in ffn_copies(j + 1):
                c.start()

        @pl.when(j == 2)
        def _():
            att_copies[0].start()

        @pl.when(j == 3)
        def _():
            att_copies[1].start()

        def row_body(r, carry2):
            ffn_tile(j, r, False)
            return carry2
        return jax.lax.fori_loop(0, nrf, row_body, carry)
    jax.lax.fori_loop(1, nf - 1, chunk_body, 0)

    for c in ffn_copies(nf - 1) + att_copies:
        c.wait()
    dh = d // _H
    wr = d // 2 // nrf
    wc = d // nrf

    def last_body(r, carry):
        ffn_tile(nf - 1, r, False)
        for b in range(wr // 128):
            rows_b = pl.ds(pl.multiple_of(r * (2 * wr) + b * 256, 256), 256)
            words = pltpu.bitcast(wqkv_v[rows_b, :], jnp.int32)
            t_s[b] = words.T
            parts = [t_s[b, pl.ds(m * d + e, _H, stride=dh), :]
                     for m in range(3) for e in range(dh)]
            wqkv_v[rows_b, :] = pltpu.bitcast(jnp.concatenate(parts, axis=0).T, jnp.bfloat16)
        for b in range(wc // 128):
            cols = pl.ds(pl.multiple_of(r * wc + b * 128, 128), 128)
            u_s[b] = wo_v[:, cols].astype(f32)
            parts = [u_s[b, pl.ds(e, _H, stride=dh), :] for e in range(dh)]
            wo_v[:, cols] = jnp.concatenate(parts, axis=0).astype(jnp.bfloat16)
        return carry
    jax.lax.fori_loop(0, nrf, last_body, 0)

    scale = np.float32((d // _H) ** -0.5)
    gw = gw_ref[...].astype(f32)

    def att_body(r, carry):
        r0 = pl.multiple_of(r * ta, ta)
        rows = pl.ds(r0, ta)
        x = x_v[rows, :]
        qk = jnp.dot(x, wqkv_v[:, :2 * d], preferred_element_type=f32)
        for c in range(nch):
            q_s[c] = qk[:, c * 128:(c + 1) * 128]
            k_s[c, pl.ds(_HALO, ta), :] = qk[:, d + c * 128: d + (c + 1) * 128]
        v = jnp.dot(x, wqkv_v[:, 2 * d:], preferred_element_type=f32)
        for c in range(nch):
            v_s[c, pl.ds(_HALO, ta), :] = v[:, c * 128:(c + 1) * 128]

        for g0 in range(0, ta, _RG):
            qs = [q_s[c, pl.ds(g0, _RG), :] for c in range(nch)]
            row = r0 + g0 + jax.lax.broadcasted_iota(jnp.int32, (_RG, 128), 0)
            logits = []
            for w in range(_W):
                s = None
                for c in range(nch):
                    p = qs[c] * k_s[c, pl.ds(_HALO + g0 - _DIL * w, _RG), :]
                    s = p if s is None else s + p
                s = s + pltpu.roll(s, 64, 1)
                s = s + pltpu.roll(s, 32, 1)
                l = s * scale
                if _DIL * w > g0:
                    l = jnp.where(row >= _DIL * w, l, np.float32(-1e9))
                logits.append(l)
            m = functools.reduce(jnp.maximum, logits)
            es = [jnp.exp(l - m) for l in logits]
            inv = 1.0 / functools.reduce(lambda a, b: a + b, es)
            for w in range(_W):
                p_s[w, pl.ds(g0, _RG), :] = es[w] * inv

        for c in range(nch):
            for g0 in range(0, ta, _RGV):
                o = None
                for w in range(_W):
                    t = p_s[w, pl.ds(g0, _RGV), :] * v_s[c, pl.ds(_HALO + g0 - _DIL * w, _RGV), :]
                    o = t if o is None else o + t
                a_s[pl.ds(g0, _RGV), c * 128:(c + 1) * 128] = o.astype(jnp.bfloat16)
        k_s[:, pl.ds(0, _HALO), :] = k_s[:, pl.ds(ta, _HALO), :]
        v_s[:, pl.ds(0, _HALO), :] = v_s[:, pl.ds(ta, _HALO), :]
        a = jnp.dot(a_s[...], wo_v[...], preferred_element_type=f32)

        g = jax.nn.sigmoid(jnp.sum(x.astype(f32) * gw, axis=-1, keepdims=True))
        out_v[rows, :] = (g * a + (1.0 - g) * acc_s[rows, :]).astype(out_v.dtype)
        out_copy(r).start()
        return carry
    jax.lax.fori_loop(0, nra, att_body, 0)
    for r in range(nra):
        out_copy(r).wait()


@jax.jit
def pallas_gated_mix__sliding_local_dilated__glu_gated_reglu__prompt_kernel(
    A_x: jax.Array,
    A_wqkv: jax.Array,
    A_wo: jax.Array,
    B_x: jax.Array,
    B_W_gate: jax.Array,
    B_W_up: jax.Array,
    B_W_down: jax.Array,
    gate_w: jax.Array,
):
    del B_x
    B, S, D = A_x.shape
    F = B_W_gate.shape[1]
    tf, ta, fc = _TF, _TA, _FC
    nf = F // fc
    nch = D // 128
    x2 = A_x.reshape(B * S, D)
    gw = gate_w.reshape(1, D)

    any_spec = pl.BlockSpec(memory_space=pl.ANY)
    bf16 = jnp.bfloat16
    out = pl.pallas_call(
        functools.partial(_kernel, S=S, d=D, tf=tf, ta=ta, fc=fc, nf=nf),
        in_specs=[
            any_spec,
            pl.BlockSpec(memory_space=pltpu.VMEM),
            any_spec, any_spec, any_spec, any_spec, any_spec,
        ],
        out_specs=any_spec,
        out_shape=jax.ShapeDtypeStruct((S, D), A_x.dtype),
        scratch_shapes=[
            pltpu.VMEM((S, D), bf16),
            pltpu.VMEM((D, 3 * D), bf16),
            pltpu.VMEM((D, D), bf16),
            pltpu.VMEM((nf, D, fc), bf16),
            pltpu.VMEM((nf, D, fc), bf16),
            pltpu.VMEM((nf, fc, D), bf16),
            pltpu.VMEM((S, D), jnp.float32),
            pltpu.VMEM((nch, ta + _HALO, 128), jnp.float32),
            pltpu.VMEM((nch, ta + _HALO, 128), jnp.float32),
            pltpu.VMEM((nch, ta, 128), jnp.float32),
            pltpu.VMEM((_W, ta, 128), jnp.float32),
            pltpu.VMEM((ta, D), bf16),
            pltpu.VMEM((S, D), A_x.dtype),
            pltpu.VMEM((D // 2 // (S // tf) // 128, 3 * D, 128), jnp.int32),
            pltpu.VMEM((D // (S // tf) // 128, D, 128), jnp.float32),
            pltpu.SemaphoreType.DMA((S // tf,)),
            pltpu.SemaphoreType.DMA((2,)),
            pltpu.SemaphoreType.DMA((3, nf)),
            pltpu.SemaphoreType.DMA((S // ta,)),
        ],
        compiler_params=pltpu.CompilerParams(
            vmem_limit_bytes=110 * 1024 * 1024,
            flags=_FLAGS,
        ),
    )(x2, gw, A_wqkv, A_wo, B_W_gate, B_W_up, B_W_down)
    return out.reshape(B, S, D)
```

```python
import functools

import jax
import jax.numpy as jnp
import numpy as np
import jax.experimental.pallas as pl
import jax.experimental.pallas.tpu as pltpu

_H = 32
_W = 8
_DIL = 2
_HALO = 16
_FLAGS = {"XLA_TPU_EVENLY_DISTRIBUTE_CRITICAL_NODES": True}
_RG = 64
_RGV = 64
_TF = 512
_TA = 512
_FC = 512


def _kernel(x_hbm, gw_ref, wqkv_hbm, wo_hbm, wg_hbm, wu_hbm, wd_hbm, o_hbm,
            x_v, wqkv_v, wo_v, wg_v, wu_v, wd_v, acc_s, k_s, v_s, q_s, p_s, a_s, out_v, t_s, u_s,
            sem_x, sem_a, sem_f, sem_o, *, S, d, tf, ta, fc, nf):
    nch = d // 128
    nrf = S // tf
    nra = S // ta
    f32 = jnp.float32

    def x_copy(r):
        return pltpu.make_async_copy(x_hbm.at[pl.ds(r * tf, tf), :],
                                     x_v.at[pl.ds(r * tf, tf), :], sem_x.at[r])

    def ffn_copies(j):
        return (
            pltpu.make_async_copy(wg_hbm.at[:, pl.ds(j * fc, fc)], wg_v.at[j], sem_f.at[0, j]),
            pltpu.make_async_copy(wu_hbm.at[:, pl.ds(j * fc, fc)], wu_v.at[j], sem_f.at[1, j]),
            pltpu.make_async_copy(wd_hbm.at[pl.ds(j * fc, fc), :], wd_v.at[j], sem_f.at[2, j]),
        )

    att_copies = (
        pltpu.make_async_copy(wqkv_hbm, wqkv_v, sem_a.at[0]),
        pltpu.make_async_copy(wo_hbm, wo_v, sem_a.at[1]),
    )

    def out_copy(r):
        return pltpu.make_async_copy(out_v.at[pl.ds(r * ta, ta), :],
                                     o_hbm.at[pl.ds(r * ta, ta), :], sem_o.at[r])

    x_copy(0).start()
    for c in ffn_copies(0):
        c.start()

    def ffn_tile(j, r, first):
        rows = pl.ds(pl.multiple_of(r * tf, tf), tf)
        x = x_v[rows, :]
        gate = jnp.dot(x, wg_v[j], preferred_element_type=f32)
        up = jnp.dot(x, wu_v[j], preferred_element_type=f32)
        h = ((gate * (gate > 0).astype(f32)) * up).astype(jnp.bfloat16)
        part = jnp.dot(h, wd_v[j], preferred_element_type=f32)
        if first:
            acc_s[rows, :] = part
        else:
            acc_s[rows, :] += part

    x_copy(0).wait()
    for c in ffn_copies(0):
        c.wait()
    for r in range(1, nrf):
        x_copy(r).start()
    for c in ffn_copies(1):
        c.start()
    k_s[:, pl.ds(0, _HALO), :] = jnp.zeros((nch, _HALO, 128), f32)
    v_s[:, pl.ds(0, _HALO), :] = jnp.zeros((nch, _HALO, 128), f32)

    def first_body(r, carry):
        @pl.when(r > 0)
        def _():
            x_copy(r).wait()
        ffn_tile(0, r, True)
        return carry
    jax.lax.fori_loop(0, nrf, first_body, 0)

    def chunk_body(j, carry):
        for c in ffn_copies(j):
            c.wait()

        @pl.when(j + 1 < nf)
        def _():
            for c in ffn_copies(j + 1):
                c.start()

        @pl.when(j == 2)
        def _():
            att_copies[0].start()

        @pl.when(j == 3)
        def _():
            att_copies[1].start()

        def row_body(r, carry2):
            ffn_tile(j, r, False)
            return carry2
        return jax.lax.fori_loop(0, nrf, row_body, carry)
    jax.lax.fori_loop(1, nf - 1, chunk_body, 0)

    for c in ffn_copies(nf - 1) + att_copies:
        c.wait()
    dh = d // _H
    wr = d // 2 // nrf
    wc = d // nrf

    def last_body(r, carry):
        ffn_tile(nf - 1, r, False)
        for b in range(wr // 128):
            rows_b = pl.ds(pl.multiple_of(r * (2 * wr) + b * 256, 256), 256)
            words = pltpu.bitcast(wqkv_v[rows_b, :], jnp.int32)
            t_s[b] = words.T
            parts = [t_s[b, pl.ds(m * d + e, _H, stride=dh), :]
                     for m in range(3) for e in range(dh)]
            wqkv_v[rows_b, :] = pltpu.bitcast(jnp.concatenate(parts, axis=0).T, jnp.bfloat16)
        for b in range(wc // 128):
            cols = pl.ds(pl.multiple_of(r * wc + b * 128, 128), 128)
            u_s[b] = wo_v[:, cols].astype(f32)
            parts = [u_s[b, pl.ds(e, _H, stride=dh), :] for e in range(dh)]
            wo_v[:, cols] = jnp.concatenate(parts, axis=0).astype(jnp.bfloat16)
        return carry
    jax.lax.fori_loop(0, nrf, last_body, 0)

    scale = np.float32((d // _H) ** -0.5)
    gw = gw_ref[...].astype(f32)

    def att_body(r, carry):
        r0 = pl.multiple_of(r * ta, ta)
        rows = pl.ds(r0, ta)
        x = x_v[rows, :]
        qk = jnp.dot(x, wqkv_v[:, :2 * d], preferred_element_type=f32)
        for c in range(nch):
            q_s[c] = qk[:, c * 128:(c + 1) * 128]
            k_s[c, pl.ds(_HALO, ta), :] = qk[:, d + c * 128: d + (c + 1) * 128]
        v = jnp.dot(x, wqkv_v[:, 2 * d:], preferred_element_type=f32)
        for c in range(nch):
            v_s[c, pl.ds(_HALO, ta), :] = v[:, c * 128:(c + 1) * 128]

        for g0 in range(0, ta, _RG):
            qs = [q_s[c, pl.ds(g0, _RG), :] for c in range(nch)]
            row = r0 + g0 + jax.lax.broadcasted_iota(jnp.int32, (_RG, 128), 0)
            sums = [None] * _W
            for w in range(_W // 2):
                for c in range(nch):
                    kk = k_s[c, pl.ds(_HALO + g0 - _DIL * w - 8, _RG + 8), :]
                    for ww, kt in ((w, kk[8:]), (w + _W // 2, kk[:_RG])):
                        p = qs[c] * kt
                        sums[ww] = p if sums[ww] is None else sums[ww] + p
            logits = []
            for w in range(_W):
                s = sums[w]
                s = s + pltpu.roll(s, 64, 1)
                s = s + pltpu.roll(s, 32, 1)
                l = s * scale
                if _DIL * w > g0:
                    l = jnp.where(row >= _DIL * w, l, np.float32(-1e9))
                logits.append(l)
            m = functools.reduce(jnp.maximum, logits)
            es = [jnp.exp(l - m) for l in logits]
            inv = 1.0 / functools.reduce(lambda a, b: a + b, es)
            for w in range(_W):
                p_s[w, pl.ds(g0, _RG), :] = es[w] * inv

        for c in range(nch):
            for g0 in range(0, ta, _RGV):
                o = None
                for w in range(_W // 2):
                    vv = v_s[c, pl.ds(_HALO + g0 - _DIL * w - 8, _RGV + 8), :]
                    t = (p_s[w, pl.ds(g0, _RGV), :] * vv[8:]
                         + p_s[w + _W // 2, pl.ds(g0, _RGV), :] * vv[:_RGV])
                    o = t if o is None else o + t
                a_s[pl.ds(g0, _RGV), c * 128:(c + 1) * 128] = o.astype(jnp.bfloat16)
        k_s[:, pl.ds(0, _HALO), :] = k_s[:, pl.ds(ta, _HALO), :]
        v_s[:, pl.ds(0, _HALO), :] = v_s[:, pl.ds(ta, _HALO), :]
        a = jnp.dot(a_s[...], wo_v[...], preferred_element_type=f32)

        g = jax.nn.sigmoid(jnp.sum(x.astype(f32) * gw, axis=-1, keepdims=True))
        out_v[rows, :] = (g * a + (1.0 - g) * acc_s[rows, :]).astype(out_v.dtype)
        out_copy(r).start()
        return carry
    jax.lax.fori_loop(0, nra, att_body, 0)
    for r in range(nra):
        out_copy(r).wait()


@jax.jit
def pallas_gated_mix__sliding_local_dilated__glu_gated_reglu__prompt_kernel(
    A_x: jax.Array,
    A_wqkv: jax.Array,
    A_wo: jax.Array,
    B_x: jax.Array,
    B_W_gate: jax.Array,
    B_W_up: jax.Array,
    B_W_down: jax.Array,
    gate_w: jax.Array,
):
    del B_x
    B, S, D = A_x.shape
    F = B_W_gate.shape[1]
    tf, ta, fc = _TF, _TA, _FC
    nf = F // fc
    nch = D // 128
    x2 = A_x.reshape(B * S, D)
    gw = gate_w.reshape(1, D)

    any_spec = pl.BlockSpec(memory_space=pl.ANY)
    bf16 = jnp.bfloat16
    out = pl.pallas_call(
        functools.partial(_kernel, S=S, d=D, tf=tf, ta=ta, fc=fc, nf=nf),
        in_specs=[
            any_spec,
            pl.BlockSpec(memory_space=pltpu.VMEM),
            any_spec, any_spec, any_spec, any_spec, any_spec,
        ],
        out_specs=any_spec,
        out_shape=jax.ShapeDtypeStruct((S, D), A_x.dtype),
        scratch_shapes=[
            pltpu.VMEM((S, D), bf16),
            pltpu.VMEM((D, 3 * D), bf16),
            pltpu.VMEM((D, D), bf16),
            pltpu.VMEM((nf, D, fc), bf16),
            pltpu.VMEM((nf, D, fc), bf16),
            pltpu.VMEM((nf, fc, D), bf16),
            pltpu.VMEM((S, D), jnp.float32),
            pltpu.VMEM((nch, ta + _HALO, 128), jnp.float32),
            pltpu.VMEM((nch, ta + _HALO, 128), jnp.float32),
            pltpu.VMEM((nch, ta, 128), jnp.float32),
            pltpu.VMEM((_W, ta, 128), jnp.float32),
            pltpu.VMEM((ta, D), bf16),
            pltpu.VMEM((S, D), A_x.dtype),
            pltpu.VMEM((D // 2 // (S // tf) // 128, 3 * D, 128), jnp.int32),
            pltpu.VMEM((D // (S // tf) // 128, D, 128), jnp.float32),
            pltpu.SemaphoreType.DMA((S // tf,)),
            pltpu.SemaphoreType.DMA((2,)),
            pltpu.SemaphoreType.DMA((3, nf)),
            pltpu.SemaphoreType.DMA((S // ta,)),
        ],
        compiler_params=pltpu.CompilerParams(
            vmem_limit_bytes=110 * 1024 * 1024,
            flags=_FLAGS,
        ),
    )(x2, gw, A_wqkv, A_wo, B_W_gate, B_W_up, B_W_down)
    return out.reshape(B, S, D)
```

```python
import functools

import jax
import jax.numpy as jnp
import numpy as np
import jax.experimental.pallas as pl
import jax.experimental.pallas.tpu as pltpu

_H = 32
_W = 8
_DIL = 2
_HALO = 16
_FLAGS = {"XLA_TPU_EVENLY_DISTRIBUTE_CRITICAL_NODES": True}
_RG = 64
_RGV = 64
_VS = 2
_TF = 512
_TA = 512
_FC = 512


def _kernel(x_hbm, gw_ref, wqkv_hbm, wo_hbm, wg_hbm, wu_hbm, wd_hbm, o_hbm,
            x_v, wqkv_v, wo_v, wg_v, wu_v, wd_v, acc_s, k_s, v_s, q_s, p_s, a_s, out_v, t_s, u_s,
            sem_x, sem_a, sem_f, sem_o, *, S, d, tf, ta, fc, nf):
    nch = d // 128
    nrf = S // tf
    nra = S // ta
    f32 = jnp.float32

    def x_copy(r):
        return pltpu.make_async_copy(x_hbm.at[pl.ds(r * tf, tf), :],
                                     x_v.at[pl.ds(r * tf, tf), :], sem_x.at[r])

    def ffn_copies(j):
        return (
            pltpu.make_async_copy(wg_hbm.at[:, pl.ds(j * fc, fc)], wg_v.at[j], sem_f.at[0, j]),
            pltpu.make_async_copy(wu_hbm.at[:, pl.ds(j * fc, fc)], wu_v.at[j], sem_f.at[1, j]),
            pltpu.make_async_copy(wd_hbm.at[pl.ds(j * fc, fc), :], wd_v.at[j], sem_f.at[2, j]),
        )

    att_copies = (
        pltpu.make_async_copy(wqkv_hbm, wqkv_v, sem_a.at[0]),
        pltpu.make_async_copy(wo_hbm, wo_v, sem_a.at[1]),
    )

    def out_copy(r):
        return pltpu.make_async_copy(out_v.at[pl.ds(r * ta, ta), :],
                                     o_hbm.at[pl.ds(r * ta, ta), :], sem_o.at[r])

    x_copy(0).start()
    for c in ffn_copies(0):
        c.start()

    def ffn_tile(j, r, first):
        rows = pl.ds(pl.multiple_of(r * tf, tf), tf)
        x = x_v[rows, :]
        gate = jnp.dot(x, wg_v[j], preferred_element_type=f32)
        up = jnp.dot(x, wu_v[j], preferred_element_type=f32)
        h = ((gate * (gate > 0).astype(f32)) * up).astype(jnp.bfloat16)
        part = jnp.dot(h, wd_v[j], preferred_element_type=f32)
        if first:
            acc_s[rows, :] = part
        else:
            acc_s[rows, :] += part

    x_copy(0).wait()
    for c in ffn_copies(0):
        c.wait()
    for r in range(1, nrf):
        x_copy(r).start()
    for c in ffn_copies(1):
        c.start()
    k_s[:, pl.ds(0, _HALO), :] = jnp.zeros((nch, _HALO, 128), f32)
    v_s[:, pl.ds(0, _HALO), :] = jnp.zeros((nch, _HALO, 128), f32)

    def first_body(r, carry):
        @pl.when(r > 0)
        def _():
            x_copy(r).wait()
        ffn_tile(0, r, True)
        return carry
    jax.lax.fori_loop(0, nrf, first_body, 0)

    def chunk_body(j, carry):
        for c in ffn_copies(j):
            c.wait()

        @pl.when(j + 1 < nf)
        def _():
            for c in ffn_copies(j + 1):
                c.start()

        @pl.when(j == 2)
        def _():
            att_copies[0].start()

        @pl.when(j == 3)
        def _():
            att_copies[1].start()

        def row_body(r, carry2):
            ffn_tile(j, r, False)
            return carry2
        return jax.lax.fori_loop(0, nrf, row_body, carry)
    jax.lax.fori_loop(1, nf - 1, chunk_body, 0)

    for c in ffn_copies(nf - 1) + att_copies:
        c.wait()
    dh = d // _H
    wr = d // 2 // nrf
    wc = d // nrf

    def last_body(r, carry):
        ffn_tile(nf - 1, r, False)
        for b in range(wr // 128):
            rows_b = pl.ds(pl.multiple_of(r * (2 * wr) + b * 256, 256), 256)
            words = pltpu.bitcast(wqkv_v[rows_b, :], jnp.int32)
            t_s[b] = words.T
            parts = [t_s[b, pl.ds(m * d + e, _H, stride=dh), :]
                     for m in range(3) for e in range(dh)]
            wqkv_v[rows_b, :] = pltpu.bitcast(jnp.concatenate(parts, axis=0).T, jnp.bfloat16)
        for b in range(wc // 128):
            cols = pl.ds(pl.multiple_of(r * wc + b * 128, 128), 128)
            u_s[b] = wo_v[:, cols].astype(f32)
            parts = [u_s[b, pl.ds(e, _H, stride=dh), :] for e in range(dh)]
            wo_v[:, cols] = jnp.concatenate(parts, axis=0).astype(jnp.bfloat16)
        return carry
    jax.lax.fori_loop(0, nrf, last_body, 0)

    scale = np.float32((d // _H) ** -0.5)
    gw = gw_ref[...].astype(f32)

    def att_body(r, carry):
        r0 = pl.multiple_of(r * ta, ta)
        rows = pl.ds(r0, ta)
        x = x_v[rows, :]
        def proj(m, c0, c1):
            y = jnp.dot(x, wqkv_v[:, m * d + c0 * 128: m * d + c1 * 128],
                        preferred_element_type=f32)
            for c in range(c0, c1):
                yc = y[:, (c - c0) * 128:(c - c0 + 1) * 128]
                if m == 0:
                    q_s[c] = yc
                else:
                    (k_s, v_s)[m - 1][c, pl.ds(_HALO, ta), :] = yc

        proj(1, 0, nch)
        proj(2, 0, _VS)
        proj(0, 0, nch)
        proj(2, _VS, nch)

        for g0 in range(0, ta, _RG):
            qs = [q_s[c, pl.ds(g0, _RG), :] for c in range(nch)]
            row = r0 + g0 + jax.lax.broadcasted_iota(jnp.int32, (_RG, 128), 0)
            sums = [None] * _W
            for w in range(_W // 2):
                for c in range(nch):
                    kk = k_s[c, pl.ds(_HALO + g0 - _DIL * w - 8, _RG + 8), :]
                    for ww, kt in ((w, kk[8:]), (w + _W // 2, kk[:_RG])):
                        p = qs[c] * kt
                        sums[ww] = p if sums[ww] is None else sums[ww] + p
            logits = []
            for w in range(_W):
                s = sums[w]
                s = s + pltpu.roll(s, 64, 1)
                s = s + pltpu.roll(s, 32, 1)
                l = s * scale
                if _DIL * w > g0:
                    l = jnp.where(row >= _DIL * w, l, np.float32(-1e9))
                logits.append(l)
            m = functools.reduce(jnp.maximum, logits)
            es = [jnp.exp(l - m) for l in logits]
            inv = 1.0 / functools.reduce(lambda a, b: a + b, es)
            for w in range(_W):
                p_s[w, pl.ds(g0, _RG), :] = es[w] * inv

        for c in range(nch):
            for g0 in range(0, ta, _RGV):
                o = None
                for w in range(_W // 2):
                    vv = v_s[c, pl.ds(_HALO + g0 - _DIL * w - 8, _RGV + 8), :]
                    t = (p_s[w, pl.ds(g0, _RGV), :] * vv[8:]
                         + p_s[w + _W // 2, pl.ds(g0, _RGV), :] * vv[:_RGV])
                    o = t if o is None else o + t
                a_s[pl.ds(g0, _RGV), c * 128:(c + 1) * 128] = o.astype(jnp.bfloat16)
        k_s[:, pl.ds(0, _HALO), :] = k_s[:, pl.ds(ta, _HALO), :]
        v_s[:, pl.ds(0, _HALO), :] = v_s[:, pl.ds(ta, _HALO), :]
        a = jnp.dot(a_s[...], wo_v[...], preferred_element_type=f32)

        g = jax.nn.sigmoid(jnp.sum(x.astype(f32) * gw, axis=-1, keepdims=True))
        out_v[rows, :] = (g * a + (1.0 - g) * acc_s[rows, :]).astype(out_v.dtype)
        out_copy(r).start()
        return carry
    jax.lax.fori_loop(0, nra, att_body, 0)
    for r in range(nra):
        out_copy(r).wait()


@jax.jit
def pallas_gated_mix__sliding_local_dilated__glu_gated_reglu__prompt_kernel(
    A_x: jax.Array,
    A_wqkv: jax.Array,
    A_wo: jax.Array,
    B_x: jax.Array,
    B_W_gate: jax.Array,
    B_W_up: jax.Array,
    B_W_down: jax.Array,
    gate_w: jax.Array,
):
    del B_x
    B, S, D = A_x.shape
    F = B_W_gate.shape[1]
    tf, ta, fc = _TF, _TA, _FC
    nf = F // fc
    nch = D // 128
    x2 = A_x.reshape(B * S, D)
    gw = gate_w.reshape(1, D)

    any_spec = pl.BlockSpec(memory_space=pl.ANY)
    bf16 = jnp.bfloat16
    out = pl.pallas_call(
        functools.partial(_kernel, S=S, d=D, tf=tf, ta=ta, fc=fc, nf=nf),
        in_specs=[
            any_spec,
            pl.BlockSpec(memory_space=pltpu.VMEM),
            any_spec, any_spec, any_spec, any_spec, any_spec,
        ],
        out_specs=any_spec,
        out_shape=jax.ShapeDtypeStruct((S, D), A_x.dtype),
        scratch_shapes=[
            pltpu.VMEM((S, D), bf16),
            pltpu.VMEM((D, 3 * D), bf16),
            pltpu.VMEM((D, D), bf16),
            pltpu.VMEM((nf, D, fc), bf16),
            pltpu.VMEM((nf, D, fc), bf16),
            pltpu.VMEM((nf, fc, D), bf16),
            pltpu.VMEM((S, D), jnp.float32),
            pltpu.VMEM((nch, ta + _HALO, 128), jnp.float32),
            pltpu.VMEM((nch, ta + _HALO, 128), jnp.float32),
            pltpu.VMEM((nch, ta, 128), jnp.float32),
            pltpu.VMEM((_W, ta, 128), jnp.float32),
            pltpu.VMEM((ta, D), bf16),
            pltpu.VMEM((S, D), A_x.dtype),
            pltpu.VMEM((D // 2 // (S // tf) // 128, 3 * D, 128), jnp.int32),
            pltpu.VMEM((D // (S // tf) // 128, D, 128), jnp.float32),
            pltpu.SemaphoreType.DMA((S // tf,)),
            pltpu.SemaphoreType.DMA((2,)),
            pltpu.SemaphoreType.DMA((3, nf)),
            pltpu.SemaphoreType.DMA((S // ta,)),
        ],
        compiler_params=pltpu.CompilerParams(
            vmem_limit_bytes=110 * 1024 * 1024,
            flags=_FLAGS,
        ),
    )(x2, gw, A_wqkv, A_wo, B_W_gate, B_W_up, B_W_down)
    return out.reshape(B, S, D)
```
